```python
import jax
import jax.numpy as jnp

def _softmax(x, axis=-1):
    return jax.nn.softmax(x, axis=axis)

def _gelu(x):
    return jax.nn.gelu(x, approximate=True)

def _silu(x):
    return jax.nn.silu(x)

def _sigmoid(x):
    return jax.nn.sigmoid(x)

def _layernorm(x, axis=-1, eps=1e-05):
    m = jnp.mean(x, axis=axis, keepdims=True)
    v = jnp.var(x, axis=axis, keepdims=True)
    return (x - m) / jnp.sqrt(v + eps)

def _scatter_add(tgt, idx, src, axis=0):
    return tgt.at[idx].add(src)

def _segment_sum(src, seg, n):
    return jax.ops.segment_sum(src, seg, n)

class _Rng:

    def __init__(self, key):
        self._k = key

    def _next(self):
        self._k, sub = jax.random.split(self._k)
        return sub

    def normal(self, shape):
        return jax.random.normal(self._next(), shape, dtype=jnp.bfloat16)

    def randint(self, lo, hi, shape):
        return jax.random.randint(self._next(), shape, lo, hi, dtype=jnp.int32)

    def uniform(self, shape, lo=0.0, hi=1.0):
        return jax.random.uniform(self._next(), shape, jnp.bfloat16, lo, hi)

    def permutation(self, n):
        return jax.random.permutation(self._next(), n)
kernel_name = 'standalone__dilated_atrous__vision'

def setup_inputs():
    _rng = _Rng(jax.random.key(int.from_bytes(__import__("os").urandom(4), "little")))
    _w = lambda a: (lambda t: t.astype(jnp.bfloat16) if jnp.issubdtype(t.dtype, jnp.floating) else t)(jnp.asarray(a))
    H = W = 384
    C = 384
    k = 1
    return {'x': _w((lambda *s: _rng.normal(s) * 0.05)(1, H, W, C)), 'w': _w((lambda *s: _rng.normal(s) * 0.05)(k, k, C, C) * (1.0 / (k * C ** 0.5)))}

def reference(x, w):
    B, H, W, C = x.shape
    k = 1
    rate = 2
    pad = (k - 1) * rate // 2
    xp = jnp.pad(x, ((0, 0), (pad, pad), (pad, pad), (0, 0)))
    out = jnp.zeros_like(x)
    for i in range(k):
        for j in range(k):
            tap = xp[:, i * rate:i * rate + H, j * rate:j * rate + W, :].copy()
            out = out + jnp.einsum('bhwc,co->bhwo', tap, w[i, j])
    return out
```

```python
import jax
import jax.numpy as jnp
import jax.experimental.pallas as pl
import jax.experimental.pallas.tpu as pltpu

_S = 8
_B = 1024
_T = 64
_TC = 2048
_KSTAR = 41
_WPR = 8


def _make_kernel(A, C, O):
    S, B, T, TC = _S, _B, _T, _TC
    nj = B // T
    nw = A * nj
    ks = TC // B
    cps = S // ks
    nc = A * cps
    kstar = min(_KSTAR, nc)

    def kernel(x_hbm, w_hbm, o_hbm, buf, wbuf, rsem, wsem, osem):
        def rd(a):
            return pltpu.make_async_copy(x_hbm.at[a], buf.at[a], rsem.at[a])

        def wr(i):
            a = i // nj
            j = pl.multiple_of((i % nj) * T, T)
            return pltpu.make_async_copy(
                buf.at[a, :, pl.ds(j, T)], o_hbm.at[a, :, pl.ds(j, T)], osem.at[0])

        wcp = pltpu.make_async_copy(w_hbm, wbuf, wsem.at[0])
        wcp.start()
        for a in range(A):
            rd(a).start(priority=1)
        wcp.wait()

        def compute(k):
            a = k // cps
            s0 = (k % cps) * ks
            v = buf[a, pl.ds(s0, ks)].reshape(TC, C)
            r = jnp.dot(v, wbuf[...], preferred_element_type=jnp.float32)
            buf[a, pl.ds(s0, ks)] = r.astype(buf.dtype).reshape(ks, B, O)

        def body1(k, c):
            @pl.when(k % cps == 0)
            def _():
                rd(k // cps).wait()
            compute(k)
            return c

        jax.lax.fori_loop(0, kstar, body1, 0)
        for a in range((kstar + cps - 1) // cps, A):
            rd(a).wait()

        def issue(i, c):
            wr(i).start()
            return c

        def body2(k, issued):
            tgt = jnp.minimum((k // cps) * nj, issued + _WPR)
            jax.lax.fori_loop(issued, tgt, issue, 0)
            compute(k)
            return tgt

        issued = jax.lax.fori_loop(kstar, nc, body2, 0)
        jax.lax.fori_loop(issued, nw, issue, 0)
        pltpu.make_async_copy(buf, o_hbm, osem.at[0]).wait()

    return kernel


@jax.jit
def pallas_standalone__dilated_atrous__vision_kernel(x: jax.Array, w: jax.Array):
    Bt, H, W, C = x.shape
    O = w.shape[-1]
    M = Bt * H * W
    assert C == O and M % (_S * _B) == 0
    A = M // (_S * _B)
    x4 = x.reshape(A, _S, _B, C)
    w2 = w.reshape(C, O)
    out = pl.pallas_call(
        _make_kernel(A, C, O),
        in_specs=[pl.BlockSpec(memory_space=pl.ANY), pl.BlockSpec(memory_space=pl.ANY)],
        out_specs=pl.BlockSpec(memory_space=pl.ANY),
        out_shape=jax.ShapeDtypeStruct((A, _S, _B, O), x.dtype),
        scratch_shapes=[
            pltpu.VMEM((A, _S, _B, C), x.dtype),
            pltpu.VMEM((C, O), w.dtype),
            pltpu.SemaphoreType.DMA((A,)),
            pltpu.SemaphoreType.DMA((1,)),
            pltpu.SemaphoreType.DMA((1,)),
        ],
        compiler_params=pltpu.CompilerParams(vmem_limit_bytes=125 * 1024 * 1024),
    )(x4, w2)
    return out.reshape(Bt, H, W, O)
```

```python
import jax
import jax.numpy as jnp
import jax.experimental.pallas as pl
import jax.experimental.pallas.tpu as pltpu

_S = 6
_B = 2048
_TR = 32
_TW = 32
_TJ = 256
_UR = 512
_PRE = 3
_EXTRA = 1
_BURST = 32
_K2 = 14


def _make_kernel(A, C, O):
    S, B = _S, _B
    Sh = S // 2
    upg = B // _UR
    nu = A * upg
    spg = B // _TJ
    ns = A * spg
    wpg = B // _TW
    nw = A * wpg
    wps = _TJ // _TW
    R = _PRE + 1
    n1 = nu - _PRE
    ksw = n1 + _EXTRA
    assert ksw < ns and _UR >= _TJ

    def kernel(x_hbm, w_hbm, o_hbm, buf, wbuf, rsem, wsem, osem):
        def issue_unit(u):
            g = u // upg
            j0 = (u % upg) * _UR
            sem = rsem.at[u % R]
            for i in range(_UR // _TR):
                j = j0 + i * _TR
                if not isinstance(j, int):
                    j = pl.multiple_of(j, _TR)
                for h in range(2):
                    pltpu.make_async_copy(
                        x_hbm.at[g, pl.ds(h * Sh, Sh), pl.ds(j, _TR)],
                        buf.at[g, pl.ds(h * Sh, Sh), pl.ds(j, _TR)],
                        sem).start(priority=h)

        def wait_unit(u):
            g = u // upg
            j0 = (u % upg) * _UR
            if not isinstance(j0, int):
                j0 = pl.multiple_of(j0, _UR)
            pltpu.make_async_copy(
                x_hbm.at[g, :, pl.ds(j0, _UR)], buf.at[g, :, pl.ds(j0, _UR)],
                rsem.at[u % R]).wait()

        def issue_write(i, c):
            g = i // wpg
            j = pl.multiple_of((i % wpg) * _TW, _TW)
            pltpu.make_async_copy(
                buf.at[g, :, pl.ds(j, _TW)], o_hbm.at[g, :, pl.ds(j, _TW)],
                osem.at[0]).start()
            return c

        def compute(k):
            g = k // spg
            j0 = pl.multiple_of((k % spg) * _TJ, _TJ)
            v = buf[g, :, pl.ds(j0, _TJ), :].reshape(S * _TJ, C)
            r = jnp.dot(v, wbuf[...], preferred_element_type=jnp.float32)
            buf[g, :, pl.ds(j0, _TJ), :] = r.astype(buf.dtype).reshape(S, _TJ, O)

        wcp = pltpu.make_async_copy(w_hbm, wbuf, wsem.at[0])
        wcp.start()
        for u in range(_PRE):
            issue_unit(u)

        def step(k, issued):
            @pl.when(k < n1)
            def _():
                issue_unit(k + _PRE)

            @pl.when(k == 0)
            def _():
                wcp.wait()
                wait_unit(0)

            @pl.when(k == ksw)
            def _():
                for u in range(n1, nu - 1):
                    wait_unit(u)

            inc = jnp.where(k == ksw, _BURST, jnp.where(k > ksw, _K2, 0))
            tgt = jnp.minimum(k * wps, issued + inc)
            jax.lax.fori_loop(issued, tgt, issue_write, 0)

            @pl.when(k == ksw)
            def _():
                wait_unit(nu - 1)

            compute(k)

            @pl.when(jnp.logical_and(k > 0, k < n1))
            def _():
                wait_unit(k)

            return tgt

        issued = jax.lax.fori_loop(0, ns, step, 0)
        jax.lax.fori_loop(issued, nw, issue_write, 0)
        pltpu.make_async_copy(buf, o_hbm, osem.at[0]).wait()

    return kernel, R


@jax.jit
def pallas_standalone__dilated_atrous__vision_kernel(x: jax.Array, w: jax.Array):
    Bt, H, W, C = x.shape
    O = w.shape[-1]
    M = Bt * H * W
    assert C == O and M % (_S * _B) == 0
    A = M // (_S * _B)
    x4 = x.reshape(A, _S, _B, C)
    w2 = w.reshape(C, O)
    kernel, R = _make_kernel(A, C, O)
    out = pl.pallas_call(
        kernel,
        in_specs=[pl.BlockSpec(memory_space=pl.ANY), pl.BlockSpec(memory_space=pl.ANY)],
        out_specs=pl.BlockSpec(memory_space=pl.ANY),
        out_shape=jax.ShapeDtypeStruct((A, _S, _B, O), x.dtype),
        scratch_shapes=[
            pltpu.VMEM((A, _S, _B, C), x.dtype),
            pltpu.VMEM((C, O), w.dtype),
            pltpu.SemaphoreType.DMA((R,)),
            pltpu.SemaphoreType.DMA((1,)),
            pltpu.SemaphoreType.DMA((1,)),
        ],
        compiler_params=pltpu.CompilerParams(
            vmem_limit_bytes=125 * 1024 * 1024, disable_bounds_checks=True),
    )(x4, w2)
    return out.reshape(Bt, H, W, O)
```

```python
import jax
import jax.numpy as jnp
from jax import lax
import jax.experimental.pallas as pl
import jax.experimental.pallas.tpu as pltpu

_S = 6
_BH = 1024
_TR = 8
_TW = 16
_T1 = 128
_T2 = 256
_PRE = 4
_FIRST_LOW = 27
_OV = 96
_BURST = 64
_K1 = 14
_K2 = 26


def _div(x, n):
    assert n > 0 and n & (n - 1) == 0
    s = n.bit_length() - 1
    return x >> s if isinstance(x, int) else lax.shift_right_logical(x, jnp.int32(s))


def _mod(x, n):
    assert n > 0 and n & (n - 1) == 0
    return x & (n - 1)


def _aligned(x, n):
    return x if isinstance(x, int) else pl.multiple_of(x, n)


def _make_kernel(A, C, O):
    S, BH, UR = _S, _BH, _T1
    upg = BH // UR
    nu = A * upg
    wph = BH // _TW
    nw = A * 2 * wph
    R = _PRE + 1
    n1 = nu - _PRE
    ksw = n1
    r21 = _T2 // _T1
    na = -(-(ksw + 1) // r21) * r21
    nb0 = na // r21
    nb = A * 2 * BH // _T2
    i0 = _BURST + (na - 1 - ksw) * _K1
    i1 = i0 + (nb - nb0) * _K2
    assert _BURST <= ksw * (_T1 // _TW) and i0 <= (na - 1) * (_T1 // _TW)
    assert all(i0 + (n + 1) * _K2 <= (nb0 + n) * (_T2 // _TW) for n in range(nb - nb0))
    assert 0 < _OV < 2 * UR and _OV % _TR == 0 and _PRE >= 2 and upg >= 2

    def kernel(x_hbm, w_hbm, o_hbm, buf, wbuf, rsem, osem):
        def issue_rows(g, j0, n, sem_of_row, n_low=0):
            for i in range(n // _TR):
                j = j0 + i * _TR
                for h in range(2):
                    rows = pl.ds(_aligned(j, _TR), _TR)
                    pltpu.make_async_copy(
                        x_hbm.at[g, :, h, rows], buf.at[g, :, h, rows], sem_of_row(j)
                    ).start(priority=1 if 2 * i + h < n_low else h)

        def wait_rows(g, j0, n, sem):
            rows = pl.ds(_aligned(j0, _TR), n)
            pltpu.make_async_copy(x_hbm.at[g, :, :, rows], buf.at[g, :, :, rows], sem).wait()

        def unit_sem(u):
            return rsem.at[u % R if isinstance(u, int) else lax.rem(u, jnp.int32(R))]

        def issue_unit(u, n_low=0):
            sem = unit_sem(u)
            issue_rows(_div(u, upg), _mod(u, upg) * UR, UR, lambda j: sem, n_low)

        def wait_unit(u):
            wait_rows(_div(u, upg), _mod(u, upg) * UR, UR, unit_sem(u))

        def issue_write(i):
            g = _div(i, 2 * wph)
            h = _mod(_div(i, wph), 2)
            rows = pl.ds(_aligned(_mod(i, wph) * _TW, _TW), _TW)
            pltpu.make_async_copy(
                buf.at[g, :, h, rows], o_hbm.at[g, :, h, rows], osem.at[0]).start()

        def matmul_step(k, t):
            sph = BH // t
            g = _div(k, 2 * sph)
            h = _mod(_div(k, sph), 2)
            rows = pl.ds(pl.multiple_of(_mod(k, sph) * t, t), t)
            v = buf[g, :, h, rows, :].reshape(S * t, C)
            r = jnp.dot(v, wbuf[...], preferred_element_type=jnp.float32)
            buf[g, :, h, rows, :] = r.astype(buf.dtype).reshape(S, t, O)

        wcp = pltpu.make_async_copy(w_hbm, wbuf, osem.at[0])
        issue_unit(0, _FIRST_LOW)
        wcp.start()

        def prologue(u, c):
            issue_unit(u)
            return c

        lax.fori_loop(1, _PRE, prologue, 0)
        wcp.wait()

        gl, jt, jb = A - 1, BH - 2 * UR, BH - _OV
        sem_a, sem_b = unit_sem(nu - 2), unit_sem(nu - 1)

        def tail_sem(j):
            return sem_a if j < jb else sem_b

        def step1(k, c):
            @pl.when(k < n1 - 2)
            def _():
                issue_unit(k + _PRE)

            @pl.when(k < n1)
            def _():
                wait_unit(k)

            @pl.when(k == n1 - 2)
            def _():
                issue_rows(gl, jt, UR, tail_sem)

            @pl.when(k == n1 - 1)
            def _():
                issue_rows(gl, jt + UR, UR, tail_sem)

            @pl.when(k == ksw)
            def _():
                for u in range(n1, nu - 2):
                    wait_unit(u)
                wait_rows(gl, jt, jb - jt, sem_a)
                for i in range(_BURST):
                    issue_write(i)
                wait_rows(gl, jb, _OV, sem_b)

            if na - 1 > ksw:
                @pl.when(k > ksw)
                def _():
                    base = _BURST + (k - ksw - 1) * _K1
                    for i in range(_K1):
                        issue_write(base + i)

            matmul_step(k, _T1)
            return c

        lax.fori_loop(0, na, step1, 0)

        def step2(k, c):
            base = i0 + (k - nb0) * _K2
            for i in range(_K2):
                issue_write(base + i)
            matmul_step(k, _T2)
            return c

        lax.fori_loop(nb0, nb, step2, 0)

        def epilogue(i, c):
            issue_write(i)
            return c

        lax.fori_loop(i1, nw, epilogue, 0)
        pltpu.make_async_copy(buf, o_hbm, osem.at[0]).wait()

    return kernel, R


@jax.jit
def pallas_standalone__dilated_atrous__vision_kernel(x: jax.Array, w: jax.Array):
    Bt, H, W, C = x.shape
    O = w.shape[-1]
    M = Bt * H * W
    assert C == O and M % (_S * 2 * _BH) == 0
    A = M // (_S * 2 * _BH)
    shape = (A, _S, 2, _BH, C)
    kernel, R = _make_kernel(A, C, O)
    out = pl.pallas_call(
        kernel,
        in_specs=[pl.BlockSpec(memory_space=pl.ANY), pl.BlockSpec(memory_space=pl.ANY)],
        out_specs=pl.BlockSpec(memory_space=pl.ANY),
        out_shape=jax.ShapeDtypeStruct(shape, x.dtype),
        scratch_shapes=[
            pltpu.VMEM(shape, x.dtype),
            pltpu.VMEM((C, O), w.dtype),
            pltpu.SemaphoreType.DMA((R,)),
            pltpu.SemaphoreType.DMA((1,)),
        ],
        compiler_params=pltpu.CompilerParams(
            vmem_limit_bytes=125 * 1024 * 1024, disable_bounds_checks=True),
    )(x.reshape(shape), w.reshape(C, O))
    return out.reshape(Bt, H, W, O)
```

```python
import jax
import jax.numpy as jnp
from jax import lax
import jax.experimental.pallas as pl
import jax.experimental.pallas.tpu as pltpu

_S = 6
_BH = 2048
_TR = 8
_TW = 16
_T1 = 128
_T2 = 256
_PRE = 4
_FIRST_LOW = 27
_OV = 96
_BURST = 64
_K1 = 14
_K2 = 28


def _div(x, n):
    assert n > 0 and n & (n - 1) == 0
    s = n.bit_length() - 1
    return x >> s if isinstance(x, int) else lax.shift_right_logical(x, jnp.int32(s))


def _mod(x, n):
    assert n > 0 and n & (n - 1) == 0
    return x & (n - 1)


def _aligned(x, n):
    return x if isinstance(x, int) else pl.multiple_of(x, n)


def _make_kernel(A, C, O):
    S, BH, UR = _S, _BH, _T1
    upg = BH // UR
    nu = A * upg
    wph = BH // _TW
    nw = A * 2 * wph
    R = _PRE + 1
    n1 = nu - _PRE
    ksw = n1
    r21 = _T2 // _T1
    na = -(-(ksw + 1) // r21) * r21
    nb0 = na // r21
    nb = A * 2 * BH // _T2
    i0 = _BURST + (na - 1 - ksw) * _K1
    i1 = i0 + (nb - nb0) * _K2
    assert _BURST <= ksw * (_T1 // _TW) and i0 <= (na - 1) * (_T1 // _TW)
    assert all(i0 + (n + 1) * _K2 <= (nb0 + n) * (_T2 // _TW) for n in range(nb - nb0))
    assert 0 < _OV < 2 * UR and _OV % _TR == 0 and _PRE >= 2 and upg >= 2

    def kernel(x_hbm, w_hbm, o_hbm, buf, wbuf, rsem, osem):
        def issue_rows(g, j0, n, sem_of_row, n_low=0):
            for i in range(n // _TR):
                j = j0 + i * _TR
                for h in range(2):
                    rows = pl.ds(_aligned(j, _TR), _TR)
                    pltpu.make_async_copy(
                        x_hbm.at[g, h, :, rows], buf.at[g, h, :, rows], sem_of_row(j)
                    ).start(priority=1 if 2 * i + h < n_low else h)

        def wait_rows(g, j0, n, sem):
            rows = pl.ds(_aligned(j0, _TR), n)
            pltpu.make_async_copy(x_hbm.at[g, :, :, rows], buf.at[g, :, :, rows], sem).wait()

        def unit_sem(u):
            return rsem.at[u % R if isinstance(u, int) else lax.rem(u, jnp.int32(R))]

        def issue_unit(u, n_low=0):
            sem = unit_sem(u)
            issue_rows(_div(u, upg), _mod(u, upg) * UR, UR, lambda j: sem, n_low)

        def wait_unit(u):
            wait_rows(_div(u, upg), _mod(u, upg) * UR, UR, unit_sem(u))

        def issue_write(i):
            g = _div(i, 2 * wph)
            h = _mod(_div(i, wph), 2)
            rows = pl.ds(_aligned(_mod(i, wph) * _TW, _TW), _TW)
            pltpu.make_async_copy(
                buf.at[g, h, :, rows], o_hbm.at[g, h, :, rows], osem.at[0]).start()

        def matmul_step(k, t):
            sph = BH // t
            g = _div(k, 2 * sph)
            h = _mod(_div(k, sph), 2)
            rows = pl.ds(pl.multiple_of(_mod(k, sph) * t, t), t)
            v = buf[g, h, :, rows, :].reshape(S * t, C)
            r = jnp.dot(v, wbuf[...], preferred_element_type=jnp.float32)
            buf[g, h, :, rows, :] = r.astype(buf.dtype).reshape(S, t, O)

        wcp = pltpu.make_async_copy(w_hbm, wbuf, osem.at[0])
        issue_unit(0, _FIRST_LOW)
        wcp.start()

        def prologue(u, c):
            issue_unit(u)
            return c

        lax.fori_loop(1, _PRE, prologue, 0)
        wcp.wait()

        gl, jt, jb = A - 1, BH - 2 * UR, BH - _OV
        sem_a, sem_b = unit_sem(nu - 2), unit_sem(nu - 1)

        def tail_sem(j):
            return sem_a if j < jb else sem_b

        def step1(k, c):
            @pl.when(k < n1 - 2)
            def _():
                issue_unit(k + _PRE)

            @pl.when(k < n1)
            def _():
                wait_unit(k)

            @pl.when(k == n1 - 2)
            def _():
                issue_rows(gl, jt, UR, tail_sem)

            @pl.when(k == n1 - 1)
            def _():
                issue_rows(gl, jt + UR, UR, tail_sem)

            @pl.when(k == ksw)
            def _():
                for u in range(n1, nu - 2):
                    wait_unit(u)
                wait_rows(gl, jt, jb - jt, sem_a)
                for i in range(_BURST):
                    issue_write(i)
                wait_rows(gl, jb, _OV, sem_b)

            if na - 1 > ksw:
                @pl.when(k > ksw)
                def _():
                    base = _BURST + (k - ksw - 1) * _K1
                    for i in range(_K1):
                        issue_write(base + i)

            matmul_step(k, _T1)
            return c

        lax.fori_loop(0, na, step1, 0)

        def step2(k, c):
            base = i0 + (k - nb0) * _K2
            for i in range(_K2):
                issue_write(base + i)
            matmul_step(k, _T2)
            return c

        lax.fori_loop(nb0, nb, step2, 0)

        def epilogue(i, c):
            issue_write(i)
            return c

        lax.fori_loop(i1, nw, epilogue, 0)
        pltpu.make_async_copy(buf, o_hbm, osem.at[0]).wait()

    return kernel, R


def _compiler_params():
    kwargs = dict(vmem_limit_bytes=125 * 1024 * 1024, disable_bounds_checks=True)
    try:
        return pltpu.CompilerParams(disable_semaphore_checks=True, **kwargs)
    except TypeError:
        return pltpu.CompilerParams(**kwargs)


@jax.jit
def pallas_standalone__dilated_atrous__vision_kernel(x: jax.Array, w: jax.Array):
    Bt, H, W, C = x.shape
    O = w.shape[-1]
    M = Bt * H * W
    assert C == O and M % (_S * 2 * _BH) == 0
    A = M // (_S * 2 * _BH)
    shape = (A, 2, _S, _BH, C)
    kernel, R = _make_kernel(A, C, O)
    out = pl.pallas_call(
        kernel,
        in_specs=[pl.BlockSpec(memory_space=pl.ANY), pl.BlockSpec(memory_space=pl.ANY)],
        out_specs=pl.BlockSpec(memory_space=pl.ANY),
        out_shape=jax.ShapeDtypeStruct(shape, x.dtype),
        scratch_shapes=[
            pltpu.VMEM(shape, x.dtype),
            pltpu.VMEM((C, O), w.dtype),
            pltpu.SemaphoreType.DMA((R,)),
            pltpu.SemaphoreType.DMA((1,)),
        ],
        compiler_params=_compiler_params(),
    )(x.reshape(shape), w.reshape(C, O))
    return out.reshape(Bt, H, W, O)
```

```python
import jax
import jax.numpy as jnp
from jax import lax
import jax.experimental.pallas as pl
import jax.experimental.pallas.tpu as pltpu

_S = 6
_SR = 3
_BH = 2048
_TR = 16
_TW = 16
_T1 = 128
_T2 = 256
_PRE = 4
_FIRST_LOW = 27
_OV = 96
_BURST = 64
_K1 = 14
_K2 = 28


def _div(x, n):
    assert n > 0 and n & (n - 1) == 0
    s = n.bit_length() - 1
    return x >> s if isinstance(x, int) else lax.shift_right_logical(x, jnp.int32(s))


def _mod(x, n):
    assert n > 0 and n & (n - 1) == 0
    return x & (n - 1)


def _aligned(x, n):
    return x if isinstance(x, int) else pl.multiple_of(x, n)


def _make_kernel(A, C, O):
    S, BH, UR = _S, _BH, _T1
    upg = BH // UR
    nu = A * upg
    wph = BH // _TW
    nw = A * 2 * wph
    R = _PRE + 1
    n1 = nu - _PRE
    ksw = n1
    r21 = _T2 // _T1
    na = -(-(ksw + 1) // r21) * r21
    nb0 = na // r21
    nb = A * 2 * BH // _T2
    i0 = _BURST + (na - 1 - ksw) * _K1
    i1 = i0 + (nb - nb0) * _K2
    assert _BURST <= ksw * (_T1 // _TW) and i0 <= (na - 1) * (_T1 // _TW)
    assert all(i0 + (n + 1) * _K2 <= (nb0 + n) * (_T2 // _TW) for n in range(nb - nb0))
    assert 0 < _OV < 2 * UR and _OV % _TR == 0 and _PRE >= 2 and upg >= 2 and S % _SR == 0

    def kernel(x_hbm, w_hbm, o_hbm, buf, wbuf, rsem, osem):
        def issue_rows(g, j0, n, sem_of_row, n_low=0):
            q = 0
            for i in range(n // _TR):
                j = j0 + i * _TR
                rows = pl.ds(_aligned(j, _TR), _TR)
                for s0 in range(0, S, _SR):
                    for h in range(2):
                        idx = (g, h, pl.ds(s0, _SR), rows)
                        pltpu.make_async_copy(
                            x_hbm.at[idx], buf.at[idx], sem_of_row(j)
                        ).start(priority=1 if q < n_low else h)
                        q += 1

        def wait_rows(g, j0, n, sem):
            rows = pl.ds(_aligned(j0, _TR), n)
            pltpu.make_async_copy(x_hbm.at[g, :, :, rows], buf.at[g, :, :, rows], sem).wait()

        def unit_sem(u):
            return rsem.at[u % R if isinstance(u, int) else lax.rem(u, jnp.int32(R))]

        def issue_unit(u, n_low=0):
            sem = unit_sem(u)
            issue_rows(_div(u, upg), _mod(u, upg) * UR, UR, lambda j: sem, n_low)

        def wait_unit(u):
            wait_rows(_div(u, upg), _mod(u, upg) * UR, UR, unit_sem(u))

        def issue_write(i):
            g = _div(i, 2 * wph)
            h = _mod(_div(i, wph), 2)
            rows = pl.ds(_aligned(_mod(i, wph) * _TW, _TW), _TW)
            pltpu.make_async_copy(
                buf.at[g, h, :, rows], o_hbm.at[g, h, :, rows], osem.at[0]).start()

        def matmul_step(k, t):
            sph = BH // t
            g = _div(k, 2 * sph)
            h = _mod(_div(k, sph), 2)
            rows = pl.ds(pl.multiple_of(_mod(k, sph) * t, t), t)
            v = buf[g, h, :, rows, :].reshape(S * t, C)
            r = jnp.dot(v, wbuf[...], preferred_element_type=jnp.float32)
            buf[g, h, :, rows, :] = r.astype(buf.dtype).reshape(S, t, O)

        wcp = pltpu.make_async_copy(w_hbm, wbuf, osem.at[0])
        issue_unit(0, _FIRST_LOW)
        wcp.start()

        def prologue(u, c):
            issue_unit(u)
            return c

        lax.fori_loop(1, _PRE, prologue, 0)
        wcp.wait()

        gl, jt, jb = A - 1, BH - 2 * UR, BH - _OV
        sem_a, sem_b = unit_sem(nu - 2), unit_sem(nu - 1)

        def tail_sem(j):
            return sem_a if j < jb else sem_b

        def step1(k, c):
            @pl.when(k < n1 - 2)
            def _():
                issue_unit(k + _PRE)

            @pl.when(k < n1)
            def _():
                wait_unit(k)

            @pl.when(k == n1 - 2)
            def _():
                issue_rows(gl, jt, UR, tail_sem)

            @pl.when(k == n1 - 1)
            def _():
                issue_rows(gl, jt + UR, UR, tail_sem)

            @pl.when(k == ksw)
            def _():
                for u in range(n1, nu - 2):
                    wait_unit(u)
                wait_rows(gl, jt, jb - jt, sem_a)
                for i in range(_BURST):
                    issue_write(i)
                wait_rows(gl, jb, _OV, sem_b)

            if na - 1 > ksw:
                @pl.when(k > ksw)
                def _():
                    base = _BURST + (k - ksw - 1) * _K1
                    for i in range(_K1):
                        issue_write(base + i)

            matmul_step(k, _T1)
            return c

        lax.fori_loop(0, na, step1, 0)

        def step2(k, c):
            base = i0 + (k - nb0) * _K2
            for i in range(_K2):
                issue_write(base + i)
            matmul_step(k, _T2)
            return c

        lax.fori_loop(nb0, nb, step2, 0)

        def epilogue(i, c):
            issue_write(i)
            return c

        lax.fori_loop(i1, nw, epilogue, 0)
        pltpu.make_async_copy(buf, o_hbm, osem.at[0]).wait()

    return kernel, R


def _compiler_params():
    kwargs = dict(vmem_limit_bytes=116 * 1024 * 1024, disable_bounds_checks=True)
    try:
        return pltpu.CompilerParams(disable_semaphore_checks=True, **kwargs)
    except TypeError:
        return pltpu.CompilerParams(**kwargs)


@jax.jit
def pallas_standalone__dilated_atrous__vision_kernel(x: jax.Array, w: jax.Array):
    Bt, H, W, C = x.shape
    O = w.shape[-1]
    M = Bt * H * W
    assert C == O and M % (_S * 2 * _BH) == 0
    A = M // (_S * 2 * _BH)
    shape = (A, 2, _S, _BH, C)
    kernel, R = _make_kernel(A, C, O)
    out = pl.pallas_call(
        kernel,
        in_specs=[pl.BlockSpec(memory_space=pl.ANY), pl.BlockSpec(memory_space=pl.ANY)],
        out_specs=pl.BlockSpec(memory_space=pl.ANY),
        out_shape=jax.ShapeDtypeStruct(shape, x.dtype),
        scratch_shapes=[
            pltpu.VMEM(shape, x.dtype),
            pltpu.VMEM((C, O), w.dtype),
            pltpu.SemaphoreType.DMA((R,)),
            pltpu.SemaphoreType.DMA((1,)),
        ],
        compiler_params=_compiler_params(),
    )(x.reshape(shape), w.reshape(C, O))
    return out.reshape(Bt, H, W, O)
```
